```python
import os as _os
_os.environ.setdefault("JAX_PLATFORMS", "cpu")
import jax
import jax.numpy as jnp

def _softmax(x, axis=-1):
    return jax.nn.softmax(x, axis=axis)
def _gelu(x):
    return jax.nn.gelu(x, approximate=True)
def _silu(x):
    return jax.nn.silu(x)
def _sigmoid(x):
    return jax.nn.sigmoid(x)
def _layernorm(x, axis=-1, eps=1e-5):
    m = jnp.mean(x, axis=axis, keepdims=True)
    v = jnp.var(x, axis=axis, keepdims=True)
    return (x - m) / jnp.sqrt(v + eps)
def _scatter_add(tgt, idx, src, axis=0):
    return tgt.at[idx].add(src)
def _segment_sum(src, seg, n):
    return jax.ops.segment_sum(src, seg, n)
class _Rng:
    def __init__(self, key):
        self._k = key
    def _next(self):
        self._k, sub = jax.random.split(self._k)
        return sub
    def normal(self, shape):
        return jax.random.normal(self._next(), shape, dtype=jnp.bfloat16)
    def randint(self, lo, hi, shape):
        return jax.random.randint(self._next(), shape, lo, hi, dtype=jnp.int32)
    def uniform(self, shape, lo=0.0, hi=1.0):
        return jax.random.uniform(self._next(), shape, jnp.bfloat16, lo, hi)
    def permutation(self, n):
        return jax.random.permutation(self._next(), n)


kernel_name = 'sequential_preLN__mha_block__moe_arch_mod__prompt'

def setup_inputs():
    _rng = _Rng(jax.random.key(int.from_bytes(__import__("os").urandom(4), "little")))
    _w = (lambda a: (lambda t: t.astype(jnp.bfloat16) if jnp.issubdtype(t.dtype, jnp.floating) else t)(jnp.asarray(a)))
    def _A_setup():
        B, S, D, H = 1, 2048, 640, 32
        return {
            "x": _w((lambda *s: _rng.normal(s) * 0.05)(B, S, D)),
            "wqkv": _w((lambda *s: _rng.normal(s) * 0.05)(D, 3 * D)),
            "wo": _w((lambda *s: _rng.normal(s) * 0.05)(D, D)),
        }
    _A_in = _A_setup()

    def _B_setup():
        B, S, D, F, C = 1, 2048, 640, 1536, 1
        return {
            "x": _w((lambda *s: _rng.normal(s) * 0.05)(B, S, D)),
            "w_r": _w((lambda *s: _rng.normal(s) * 0.05)(D)),
            "w_gate": _w((lambda *s: _rng.normal(s) * 0.05)(D, F)),
            "w_up": _w((lambda *s: _rng.normal(s) * 0.05)(D, F)),
            "w_down": _w((lambda *s: _rng.normal(s) * 0.05)(F, D)),
        }
    _B_in = _B_setup()

    return {
        "A_x": _A_in["x"],
        "A_wqkv": _A_in["wqkv"],
        "A_wo": _A_in["wo"],
        "B_x": _B_in["x"],
        "B_w_r": _B_in["w_r"],
        "B_w_gate": _B_in["w_gate"],
        "B_w_up": _B_in["w_up"],
        "B_w_down": _B_in["w_down"],
    }

def reference(A_x, A_wqkv, A_wo, B_x, B_w_r, B_w_gate, B_w_up, B_w_down):
    def _A_ref(x, wqkv, wo):
        B, S, D = x.shape
        H = 32
        Dh = D // H
        qkv = (lambda x, *d: x.transpose(*d))((x @ wqkv).reshape(B, S, 3, H, Dh), 2, 0, 3, 1, 4)
        q, k, v = qkv[0], qkv[1], qkv[2]
        scores = jnp.einsum("bhqd,bhkd->bhqk", q, k) * (Dh ** -0.5)
        p = _softmax(scores, axis=-1)
        o = jnp.einsum("bhqk,bhkd->bhqd", p, v)
        return (lambda x, *d: x.transpose(*d))(o, 0, 2, 1, 3).reshape(B, S, D) @ wo

    def _B_ref(x, w_r, w_gate, w_up, w_down):
        B, S, D = x.shape
        C = 1
        r = x @ w_r
        idx = jnp.argsort(-r, axis=-1)[:, :C]
        idx_e = jnp.repeat(idx.reshape(B, C, 1), D, axis=2)
        x_sel = jnp.take_along_axis(x, idx_e, axis=1)
        g = _silu(x_sel @ w_gate)
        u = x_sel @ w_up
        y = (g * u) @ w_down
        r_sel = _sigmoid(jnp.take_along_axis(r, idx, axis=1))
        y = y * r_sel.reshape(B, C, 1)
        b_off = (jnp.arange(B) * S).reshape(B, 1)
        flat_idx = (idx + b_off).reshape(B * C)
        zero = (x * 0.0).reshape(B * S, D)
        upd = _scatter_add(zero, flat_idx, y.reshape(B * C, D), axis=0)
        return x + upd.reshape(B, S, D)

    x = A_x
    h = x + _A_ref(_layernorm(x, axis=-1), A_wqkv, A_wo)
    h2 = h + _B_ref(_layernorm(h, axis=-1), B_w_r, B_w_gate, B_w_up, B_w_down)
    return h2
```

```python
import functools

import jax
import jax.numpy as jnp
from jax import lax
import jax.experimental.pallas as pl
import jax.experimental.pallas.tpu as pltpu

H = 32
DH = 20
HPB = 6
NB = 6
LANES = 128
EPS = 1e-5


def _ln(x):
    m = jnp.mean(x, axis=-1, keepdims=True)
    xc = x - m
    v = jnp.mean(xc * xc, axis=-1, keepdims=True)
    return xc * lax.rsqrt(v + EPS)


def _kernel(x_ref, wq_ref, wk_ref, wv_ref, wo_ref, wr_ref, wg_ref, wu_ref, wd_ref,
            o_ref,
            q_s, kt_s, v_s, h_s, best_v, best_i,
            *, S, D, TQ):
    nq = S // TQ

    xn = _ln(x_ref[...].astype(jnp.float32)).astype(jnp.bfloat16)
    q = jnp.dot(xn, wq_ref[...], preferred_element_type=jnp.float32)
    q_s[...] = (q * (DH ** -0.5)).astype(jnp.bfloat16)
    kt = lax.dot_general(wk_ref[...], xn, (((0,), (1,)), ((), ())),
                         preferred_element_type=jnp.float32)
    kt_s[...] = kt.astype(jnp.bfloat16)
    v = jnp.dot(xn, wv_ref[...], preferred_element_type=jnp.float32)
    lane = lax.broadcasted_iota(jnp.int32, v.shape, 1)
    v = jnp.where((lane % LANES) == HPB * DH, 1.0, v)
    v_s[...] = v.astype(jnp.bfloat16)

    best_v[0] = jnp.float32(-jnp.inf)
    best_i[0] = jnp.int32(0)

    lane128 = lax.broadcasted_iota(jnp.int32, (TQ, LANES), 1)

    def qblock(qi, carry):
        r0 = pl.multiple_of(qi * TQ, TQ)
        o_parts = []
        for b in range(NB):
            qb = q_s[pl.ds(r0, TQ), b * LANES:(b + 1) * LANES]
            ktb = kt_s[b * LANES:(b + 1) * LANES, :]
            vb = v_s[:, b * LANES:(b + 1) * LANES]
            nh = min(HPB, H - b * HPB)

            def head(j, acc):
                lo = j * DH
                hm = (lane128 >= lo) & (lane128 < lo + DH)
                qm = jnp.where(hm, qb, jnp.zeros_like(qb))
                s = jnp.dot(qm, ktb, preferred_element_type=jnp.float32)
                m = jnp.max(s, axis=-1, keepdims=True)
                p = jnp.exp(s - m).astype(jnp.bfloat16)
                ob = jnp.dot(p, vb, preferred_element_type=jnp.float32)
                denom = ob[:, HPB * DH:HPB * DH + 1]
                return jnp.where(hm, ob / denom, acc)

            acc = lax.fori_loop(0, nh, head, jnp.zeros((TQ, LANES), jnp.float32))
            o_parts.append(acc.astype(jnp.bfloat16))
        o = jnp.concatenate(o_parts, axis=-1)
        attn = jnp.dot(o, wo_ref[...], preferred_element_type=jnp.float32)
        h = x_ref[pl.ds(r0, TQ), :].astype(jnp.float32) + attn
        h_s[pl.ds(r0, TQ), :] = h
        x2 = _ln(h)
        o_ref[pl.ds(r0, TQ), :] = (h + x2).astype(o_ref.dtype)
        r = jnp.sum(x2 * wr_ref[...].astype(jnp.float32), axis=-1, keepdims=True)
        rmax = jnp.max(r)
        rows = lax.broadcasted_iota(jnp.int32, (TQ, 1), 0) + r0
        ridx = jnp.min(jnp.where(r == rmax, rows, S))

        @pl.when(rmax > best_v[0])
        def _():
            best_v[0] = rmax
            best_i[0] = ridx

        return carry

    lax.fori_loop(0, nq, qblock, 0)

    idx = best_i[0]
    rsel = best_v[0]
    base = pl.multiple_of((idx // 16) * 16, 16)
    hch = h_s[pl.ds(base, 16), :]
    rows16 = lax.broadcasted_iota(jnp.int32, (16, D), 0) + base
    sel = rows16 == idx
    x2c = _ln(hch)
    xb = x2c.astype(jnp.bfloat16)
    g = jnp.dot(xb, wg_ref[...], preferred_element_type=jnp.float32)
    u = jnp.dot(xb, wu_ref[...], preferred_element_type=jnp.float32)
    act = (g * jax.nn.sigmoid(g) * u).astype(jnp.bfloat16)
    y = jnp.dot(act, wd_ref[...], preferred_element_type=jnp.float32)
    gate = 1.0 / (1.0 + jnp.exp(-rsel))
    newrows = hch + x2c + jnp.where(sel, y * gate, 0.0)
    o_ref[pl.ds(base, 16), :] = newrows.astype(o_ref.dtype)


def _pad_heads_cols(w):
    d = w.shape[0]
    w = w.reshape(d, H, DH)
    w = jnp.pad(w, ((0, 0), (0, NB * HPB - H), (0, 0)))
    w = w.reshape(d, NB, HPB * DH)
    w = jnp.pad(w, ((0, 0), (0, 0), (0, LANES - HPB * DH)))
    return w.reshape(d, NB * LANES)


@jax.jit
def pallas_sequential_preLN__mha_block__moe_arch_mod__prompt_kernel(
    A_x: jax.Array,
    A_wqkv: jax.Array,
    A_wo: jax.Array,
    B_x: jax.Array,
    B_w_r: jax.Array,
    B_w_gate: jax.Array,
    B_w_up: jax.Array,
    B_w_down: jax.Array,
):
    B, S, D = A_x.shape
    TQ = 256
    x = A_x.reshape(S, D)
    wq = _pad_heads_cols(A_wqkv[:, 0:D])
    wk = _pad_heads_cols(A_wqkv[:, D:2 * D])
    wv = _pad_heads_cols(A_wqkv[:, 2 * D:3 * D])
    wo = _pad_heads_cols(A_wo.T).T
    wr = B_w_r.reshape(1, D)

    kernel = functools.partial(_kernel, S=S, D=D, TQ=TQ)
    out = pl.pallas_call(
        kernel,
        out_shape=jax.ShapeDtypeStruct((S, D), A_x.dtype),
        scratch_shapes=[
            pltpu.VMEM((S, NB * LANES), jnp.bfloat16),
            pltpu.VMEM((NB * LANES, S), jnp.bfloat16),
            pltpu.VMEM((S, NB * LANES), jnp.bfloat16),
            pltpu.VMEM((S, D), jnp.float32),
            pltpu.SMEM((1,), jnp.float32),
            pltpu.SMEM((1,), jnp.int32),
        ],
        compiler_params=pltpu.CompilerParams(vmem_limit_bytes=100 * 1024 * 1024),
    )(x, wq, wk, wv, wo, wr, B_w_gate, B_w_up, B_w_down)
    return out.reshape(B, S, D)
```

```python
import functools

import jax
import jax.numpy as jnp
from jax import lax
import jax.experimental.pallas as pl
import jax.experimental.pallas.tpu as pltpu

H = 32
DH = 20
HPB = 6
NB = 6
LANES = 128
HW = HPB * DH
EPS = 1e-5


def _ln(x):
    m = jnp.mean(x, axis=-1, keepdims=True)
    xc = x - m
    v = jnp.mean(xc * xc, axis=-1, keepdims=True)
    return xc * lax.rsqrt(v + EPS)


def _pad_cols(w_ref, off, D):
    parts = []
    for b in range(NB):
        lo = b * HW
        n = min(HW, D - lo)
        blk = w_ref[:, off + lo:off + lo + n]
        parts.append(blk)
        parts.append(jnp.zeros((w_ref.shape[0], LANES - n), w_ref.dtype))
    return jnp.concatenate(parts, axis=1)


def _kernel(x_ref, wqkv_ref, wo_ref, wr_ref, wg_hbm, wu_hbm, wd_hbm,
            o_ref,
            q_s, kt_s, v_s, h_s, w_s, wo_s, wg_ref, wu_ref, wd_ref, sems, best_v, best_i,
            *, S, D, TQ):
    nq = S // TQ

    ffn_copies = [
        pltpu.make_async_copy(wg_hbm, wg_ref, sems.at[0]),
        pltpu.make_async_copy(wu_hbm, wu_ref, sems.at[1]),
        pltpu.make_async_copy(wd_hbm, wd_ref, sems.at[2]),
    ]
    for c in ffn_copies:
        c.start()

    w_s[...] = jnp.zeros_like(w_s)
    wo_s[...] = jnp.zeros_like(wo_s)
    for t in range(3):
        for b in range(NB):
            lo = b * HW
            n = min(HW, D - lo)
            c0 = (t * NB + b) * LANES
            w_s[:, c0:c0 + n] = wqkv_ref[:, t * D + lo:t * D + lo + n]
    for b in range(NB):
        lo = b * HW
        n = min(HW, D - lo)
        wo_s[b * LANES:b * LANES + n, :] = wo_ref[lo:lo + n, :]
    NP = NB * LANES
    xn = _ln(x_ref[...].astype(jnp.float32)).astype(jnp.bfloat16)
    q = jnp.dot(xn, w_s[:, 0:NP], preferred_element_type=jnp.float32)
    q_s[...] = (q * (DH ** -0.5)).astype(jnp.bfloat16)
    kt = lax.dot_general(w_s[:, NP:2 * NP], xn, (((0,), (1,)), ((), ())),
                         preferred_element_type=jnp.float32)
    kt_s[...] = kt.astype(jnp.bfloat16)
    v = jnp.dot(xn, w_s[:, 2 * NP:3 * NP], preferred_element_type=jnp.float32)
    lane = lax.broadcasted_iota(jnp.int32, v.shape, 1)
    v = jnp.where((lane % LANES) == HW, 1.0, v)
    v_s[...] = v.astype(jnp.bfloat16)

    best_v[0] = jnp.float32(-jnp.inf)
    best_i[0] = jnp.int32(0)

    lane128 = lax.broadcasted_iota(jnp.int32, (TQ, LANES), 1)

    def qblock(qi, carry):
        r0 = pl.multiple_of(qi * TQ, TQ)
        o_parts = []
        for b in range(NB):
            qb = q_s[pl.ds(r0, TQ), b * LANES:(b + 1) * LANES]
            ktb = kt_s[b * LANES:(b + 1) * LANES, :]
            vb = v_s[:, b * LANES:(b + 1) * LANES]
            nh = min(HPB, H - b * HPB)

            def head(j, acc):
                lo = j * DH
                hm = (lane128 >= lo) & (lane128 < lo + DH)
                qm = jnp.where(hm, qb, jnp.zeros_like(qb))
                s = jnp.dot(qm, ktb, preferred_element_type=jnp.float32)
                m = jnp.max(s, axis=-1, keepdims=True)
                p = jnp.exp(s - m).astype(jnp.bfloat16)
                ob = jnp.dot(p, vb, preferred_element_type=jnp.float32)
                denom = ob[:, HW:HW + 1]
                return jnp.where(hm, ob / denom, acc)

            acc = jnp.zeros((TQ, LANES), jnp.float32)
            for j in range(nh):
                acc = head(j, acc)
            o_parts.append(acc.astype(jnp.bfloat16))
        o = jnp.concatenate(o_parts, axis=-1)
        attn = jnp.dot(o, wo_s[...], preferred_element_type=jnp.float32)
        h = x_ref[pl.ds(r0, TQ), :].astype(jnp.float32) + attn
        h_s[pl.ds(r0, TQ), :] = h
        x2 = _ln(h)
        o_ref[pl.ds(r0, TQ), :] = (h + x2).astype(o_ref.dtype)
        r = jnp.sum(x2 * wr_ref[...].astype(jnp.float32), axis=-1, keepdims=True)
        rmax = jnp.max(r)
        rows = lax.broadcasted_iota(jnp.int32, (TQ, 1), 0) + r0
        ridx = jnp.min(jnp.where(r == rmax, rows, S))

        @pl.when(rmax > best_v[0])
        def _():
            best_v[0] = rmax
            best_i[0] = ridx

        return carry

    lax.fori_loop(0, nq, qblock, 0)

    for c in ffn_copies:
        c.wait()
    idx = jnp.minimum(best_i[0], S - 1)
    rsel = best_v[0]
    base = pl.multiple_of((idx // 16) * 16, 16)
    hch = h_s[pl.ds(base, 16), :]
    rows16 = lax.broadcasted_iota(jnp.int32, (16, D), 0) + base
    sel = rows16 == idx
    x2c = _ln(hch)
    xb = x2c.astype(jnp.bfloat16)
    g = jnp.dot(xb, wg_ref[...], preferred_element_type=jnp.float32)
    u = jnp.dot(xb, wu_ref[...], preferred_element_type=jnp.float32)
    act = (g * jax.nn.sigmoid(g) * u).astype(jnp.bfloat16)
    y = jnp.dot(act, wd_ref[...], preferred_element_type=jnp.float32)
    gate = 1.0 / (1.0 + jnp.exp(-rsel))
    newrows = hch + x2c + jnp.where(sel, y * gate, 0.0)
    o_ref[pl.ds(base, 16), :] = newrows.astype(o_ref.dtype)


@jax.jit
def pallas_sequential_preLN__mha_block__moe_arch_mod__prompt_kernel(
    A_x: jax.Array,
    A_wqkv: jax.Array,
    A_wo: jax.Array,
    B_x: jax.Array,
    B_w_r: jax.Array,
    B_w_gate: jax.Array,
    B_w_up: jax.Array,
    B_w_down: jax.Array,
):
    B, S, D = A_x.shape
    TQ = 1024
    x = A_x.reshape(S, D)
    wr = B_w_r.reshape(1, D)

    kernel = functools.partial(_kernel, S=S, D=D, TQ=TQ)
    out = pl.pallas_call(
        kernel,
        out_shape=jax.ShapeDtypeStruct((S, D), A_x.dtype),
        in_specs=[
            pl.BlockSpec(memory_space=pltpu.VMEM),
            pl.BlockSpec(memory_space=pltpu.VMEM),
            pl.BlockSpec(memory_space=pltpu.VMEM),
            pl.BlockSpec(memory_space=pltpu.VMEM),
            pl.BlockSpec(memory_space=pl.ANY),
            pl.BlockSpec(memory_space=pl.ANY),
            pl.BlockSpec(memory_space=pl.ANY),
        ],
        scratch_shapes=[
            pltpu.VMEM((S, NB * LANES), jnp.bfloat16),
            pltpu.VMEM((NB * LANES, S), jnp.bfloat16),
            pltpu.VMEM((S, NB * LANES), jnp.bfloat16),
            pltpu.VMEM((S, D), jnp.float32),
            pltpu.VMEM((D, 3 * NB * LANES), jnp.bfloat16),
            pltpu.VMEM((NB * LANES, D), jnp.bfloat16),
            pltpu.VMEM(B_w_gate.shape, B_w_gate.dtype),
            pltpu.VMEM(B_w_up.shape, B_w_up.dtype),
            pltpu.VMEM(B_w_down.shape, B_w_down.dtype),
            pltpu.SemaphoreType.DMA((3,)),
            pltpu.SMEM((1,), jnp.float32),
            pltpu.SMEM((1,), jnp.int32),
        ],
        compiler_params=pltpu.CompilerParams(vmem_limit_bytes=100 * 1024 * 1024),
    )(x, A_wqkv, A_wo, wr, B_w_gate, B_w_up, B_w_down)
    return out.reshape(B, S, D)
```
